```python
import os as _os
_os.environ.setdefault("JAX_PLATFORMS", "cpu")
import jax
import jax.numpy as jnp

def _softmax(x, axis=-1):
    return jax.nn.softmax(x, axis=axis)
def _gelu(x):
    return jax.nn.gelu(x, approximate=True)
def _silu(x):
    return jax.nn.silu(x)
def _sigmoid(x):
    return jax.nn.sigmoid(x)
def _layernorm(x, axis=-1, eps=1e-5):
    m = jnp.mean(x, axis=axis, keepdims=True)
    v = jnp.var(x, axis=axis, keepdims=True)
    return (x - m) / jnp.sqrt(v + eps)
def _scatter_add(tgt, idx, src, axis=0):
    return tgt.at[idx].add(src)
def _segment_sum(src, seg, n):
    return jax.ops.segment_sum(src, seg, n)
class _Rng:
    def __init__(self, key):
        self._k = key
    def _next(self):
        self._k, sub = jax.random.split(self._k)
        return sub
    def normal(self, shape):
        return jax.random.normal(self._next(), shape, dtype=jnp.bfloat16)
    def randint(self, lo, hi, shape):
        return jax.random.randint(self._next(), shape, lo, hi, dtype=jnp.int32)
    def uniform(self, shape, lo=0.0, hi=1.0):
        return jax.random.uniform(self._next(), shape, jnp.bfloat16, lo, hi)
    def permutation(self, n):
        return jax.random.permutation(self._next(), n)


kernel_name = 'sequential_preLN__sliding_local_dilated__dense_activation_mish__prompt'

def setup_inputs():
    _rng = _Rng(jax.random.key(int.from_bytes(__import__("os").urandom(4), "little")))
    _w = (lambda a: (lambda t: t.astype(jnp.bfloat16) if jnp.issubdtype(t.dtype, jnp.floating) else t)(jnp.asarray(a)))
    def _A_setup():
        B, S, D = 1, 2048, 512
        return {
            "x": _w((lambda *s: _rng.normal(s) * 0.05)(B, S, D)),
            "wqkv": _w((lambda *s: _rng.normal(s) * 0.05)(D, 3 * D)),
            "wo": _w((lambda *s: _rng.normal(s) * 0.05)(D, D)),
        }
    _A_in = _A_setup()

    def _B_setup():
        B, S, D, F = 1, 2048, 512, 1376
        return {
            "x": _w((lambda *s: _rng.normal(s) * 0.05)(B, S, D)),
            "w1": _w((lambda *s: _rng.normal(s) * 1.6)(D, F) * (D ** -0.5)),
            "b1": _w((lambda *s: _rng.normal(s) * 0.1)(F)),
            "w2": _w((lambda *s: _rng.normal(s) * 0.1)(F, D) * (F ** -0.5)),
        }
    _B_in = _B_setup()

    return {
        "A_x": _A_in["x"],
        "A_wqkv": _A_in["wqkv"],
        "A_wo": _A_in["wo"],
        "B_x": _B_in["x"],
        "B_w1": _B_in["w1"],
        "B_b1": _B_in["b1"],
        "B_w2": _B_in["w2"],
    }

def reference(A_x, A_wqkv, A_wo, B_x, B_w1, B_b1, B_w2):
    def _A_ref(x, wqkv, wo):
        B, S, D = x.shape
        H = 32; Dh = D // H
        W, dil = 8, 2
        qkv = (lambda x, *d: x.transpose(*d))((x @ wqkv).reshape(B, S, 3, H, Dh), 2, 0, 3, 1, 4)
        q, k, v = qkv[0], qkv[1], qkv[2]
        scale = Dh ** -0.5
        pos = jnp.arange(S)
        off = jnp.arange(W) * dil
        idx = pos[:, None] - off[None, :]
        mask = idx >= 0
        idx_c = jnp.where(mask, idx, 0).reshape(-1)
        kg = k[:, :, idx_c, :].reshape(B, H, S, W, Dh)
        vg = v[:, :, idx_c, :].reshape(B, H, S, W, Dh)
        logits = jnp.einsum("bhsd,bhswd->bhsw", q, kg) * scale
        logits = jnp.where(mask[None, None, :, :], logits, -1e9)
        attn = _softmax(logits, axis=-1)
        o = jnp.einsum("bhsw,bhswd->bhsd", attn, vg)
        return (lambda x, *d: x.transpose(*d))(o, 0, 2, 1, 3).reshape(B, S, D) @ wo

    def _B_ref(x, w1, b1, w2):
        h = jnp.einsum("bsd,df->bsf", x, w1) + b1
        sp = jnp.log1p(jnp.exp(-jnp.abs(h))) + jnp.where(h > 0, h, jnp.zeros_like(h))
        act = h * jnp.tanh(sp)
        return jnp.einsum("bsf,fd->bsd", act, w2)

    x = A_x
    h = x + _A_ref(_layernorm(x, axis=-1), A_wqkv, A_wo)
    h2 = h + _B_ref(_layernorm(h, axis=-1), B_w1, B_b1, B_w2)
    return h2
```

```python
import functools
import jax
import jax.numpy as jnp
import numpy as np
from jax import lax
from jax.experimental import pallas as pl
from jax.experimental.pallas import tpu as pltpu

S, D, F, FP = 2048, 512, 1376, 1408
NG = 4
LOG2E = 1.4426950408889634
EPS = 1e-5
NT = (((1,), (1,)), ((), ()))
NXC = 8
def E(name, default=None):
    return default


FLAGS = {'XLA_TPU_RESCHEDULE_DMA_DONES': True}
if int(E('EV', 0)):
    FLAGS['XLA_TPU_EVENLY_DISTRIBUTE_CRITICAL_NODES'] = True
PINL = [int(E("PIN0", 0)), int(E("PIN1", 10))]
SPLIT = int(E("SPLIT", 1))
TREE = int(E("TREE", 0))
TREE = int(E("TREE", 1))
TL = int(E("TL", 32))
XLUP = [(int(v[0]), int(v[1])) for v in E('XLUP', '02,10,11,12,20,21,22,30,31,32').split(',') if v]
XPIN = int(E('XPIN', 6))


def _ln(x):
    m = jnp.mean(x, axis=-1, keepdims=True)
    xc = x - m
    v = jnp.mean(xc * xc, axis=-1, keepdims=True)
    return xc * jnp.exp2(-0.5 * jnp.log2(v + EPS))


def _lo(w):
    return pltpu.bitcast(w << 16, jnp.float32)


def _hi(w):
    return pltpu.bitcast(w & jnp.uint32(0xFFFF0000), jnp.float32)


def _mish(h):
    e = jnp.exp2(jnp.minimum(h * LOG2E, 20.0 * LOG2E))
    n = e * (e + 2.0)
    d = n + 2.0
    r = pl.reciprocal(d, approx=True)
    return (h * n) * r


def interleave(*gens_and_weights):
    gens = [[g, n, 0] for g, n in gens_and_weights]
    while gens:
        gens.sort(key=lambda e: (e[2] + 0.5) / e[1])
        e = gens[0]
        try:
            next(e[0])
            e[2] += 1
        except StopIteration:
            gens.remove(e)


def _pack(v):
    return pltpu.bitcast(v, jnp.uint32)


def _ld(ref, r0, n):
    return jnp.concatenate(
        [pltpu.bitcast(ref[c, pl.ds(r0 // 2, n // 2), :], jnp.bfloat16) for c in range(4)], axis=1)


def _st(ref, r0, v):
    for c in range(4):
        ref[c, pl.ds(r0 // 2, v.shape[0] // 2), :] = _pack(v[:, c * 128:(c + 1) * 128])


def kernel(x_hbm, wqkv_hbm, wo_hbm, w1_hbm, b1_hbm, w2_hbm, out_hbm,
           xbuf, wqb, wob, w1b, w2b, b1b, b1f, xn, xw, pm, wt, wop,
           kb, vb, o, outw, ybuf, abuf, wtmp,
           sem_in, sem_out, zsem):
    RC = S // NXC
    ANCH = int(E('ANCH', 1))
    ANB = int(E('ANB', 0))
    bf = jnp.bfloat16
    zs = pl.semaphore_read(zsem.at[0])
    pend = []
    pin_no = [0]

    def apply_pins(lhs, cost=1):
        for e in pend:
            e[0] -= cost
        due = [e for e in pend if e[0] <= 0]
        for e in due:
            pend.remove(e)
            pin_no[0] += 1
            zv = jnp.full((8, 128), zs * pin_no[0], jnp.int32).astype(jnp.uint32)
            first = pltpu.bitcast(pltpu.bitcast(lhs[0:16, 0:128], jnp.uint32) | (e[1] & zv), lhs.dtype)
            top = jnp.concatenate([first, lhs[0:16, 128:]], axis=1) if lhs.shape[1] > 128 else first
            lhs = jnp.concatenate([top, lhs[16:]], axis=0)
        return lhs

    kvres = []
    last = {}

    def after(v):
        return pltpu.bitcast(v, jnp.int32)[0, 0] & zs

    def x_copy(c, cc, z=0):
        return pltpu.make_async_copy(
            x_hbm.at[pl.ds(c * RC, RC), pl.ds(cc * 128, 128)],
            xbuf.at[cc].bitcast(bf).at[pl.ds(c * RC, RC), :], sem_in.at[z + c * 4 + cc])

    def wq_copy(s, z=0):
        return pltpu.make_async_copy(
            wqkv_hbm.at[:, pl.ds(s * 128, 128)], wqb.at[s].bitcast(bf), sem_in.at[z + 32 + s])

    def wo_copy(s, z=0):
        return pltpu.make_async_copy(
            wo_hbm.at[:, pl.ds(s * 128, 128)], wob.at[s].bitcast(bf), sem_in.at[z + 44 + s])

    def w1_copy(s, z=0):
        return pltpu.make_async_copy(
            w1_hbm.at[:, pl.ds(s * 128, 128)], w1b.at[s].bitcast(bf).at[pl.ds(0, F), :], sem_in.at[z + 48 + s])

    def w2_copy(s, z=0):
        return pltpu.make_async_copy(
            w2_hbm.at[:, pl.ds(s * 128, 128)], w2b.at[s].bitcast(bf).at[pl.ds(0, F), :], sem_in.at[z + 52 + s])

    def b1_copy(z=0):
        return pltpu.make_async_copy(b1_hbm, b1b, sem_in.at[z + 56])

    def out_copy(t, cc):
        return pltpu.make_async_copy(
            outw.at[cc].bitcast(bf).at[pl.ds(t * 256 if isinstance(t, int) else pl.multiple_of(t * 256, 256), 256), :],
            out_hbm.at[pl.ds(t * 256 if isinstance(t, int) else pl.multiple_of(t * 256, 256), 256), pl.ds(cc * 128, 128)],
            sem_out.at[t, cc])

    for t in (1, 2):
        wq_copy(4 * t).start()
    for c in range(NXC // 2):
        for cc in range(4):
            x_copy(c, cc).start()
    for t in (1, 2, 0):
        wq_copy(4 * t + 1).start()
    wq_copy(0).start()
    for c in range(NXC // 2, NXC):
        for cc in range(4):
            x_copy(c, cc).start()
    for g in range(2, NG):
        for t in (1, 2, 0):
            wq_copy(4 * t + g).start()
    for s in range(4):
        wo_copy(s).start()
    b1_copy().start()
    for s in range(4):
        w1_copy(s).start()
    for s in range(4):
        w2_copy(s).start()

    for s in range(4):
        w1b[s, pl.ds(F // 2, (FP - F) // 2), :] = jnp.zeros(((FP - F) // 2, 128), jnp.uint32)
        w2b[s, pl.ds(F // 2, (FP - F) // 2), :] = jnp.zeros(((FP - F) // 2, 128), jnp.uint32)

    rho = lax.broadcasted_iota(jnp.int32, (128, 128), 0)
    fi = lax.broadcasted_iota(jnp.int32, (128, 128), 1)
    pm[...] = _pack(jnp.where(fi == 16 * (rho % 8) + rho // 8, 1.0, 0.0).astype(bf))

    def prep_wt(g, t):
        s = 4 * ((t + 1) % 3) + g
        if (g, t) in XLUP:
            for dt in range(4):
                tmp = wtmp.at[s * 4 + dt]
                tmp[...] = _pack(pltpu.bitcast(wqb[s, pl.ds(64 * dt, 64), :], bf).T)
                parts = []
                for j in range(8):
                    w = tmp[pl.ds(j, 8, stride=8), :]
                    parts += [_lo(w), _hi(w)]
                wt[dt, pl.ds((g * 384 + t * 128) // 2, 64), :] = _pack(jnp.concatenate(parts, axis=0).astype(bf))
                if dt == 3 and XPIN:
                    pend.append([XPIN, wt[dt, pl.ds((g * 384 + t * 128) // 2, 8), :]])
            return
        r = lax.dot_general(pltpu.bitcast(pm[...], bf), pltpu.bitcast(wqb[s], bf), NT,
                            preferred_element_type=jnp.float32)
        _st(wt, g * 384 + t * 128, r.astype(bf))

    def prep_wo():
        for s in range(4):
            for g in range(NG):
                parts = []
                for j in range(8):
                    w = wob[s, pl.ds(g * 64 + j, 8, stride=8), :]
                    parts += [_lo(w), _hi(w)]
                wop[s, pl.ds(g * 64, 64), :] = _pack(jnp.concatenate(parts, axis=0).astype(bf))
                yield
    N_PREP_WO = 16

    def ln1_chunk(c, pin=0):
        nl = RC // 16
        for i in range(8):
            words = [xbuf[cc, pl.ds(c * RC // 2 + i, nl, stride=8), :] for cc in range(4)]
            for cc in range(4):
                xw[i, pl.ds(c * nl, nl), pl.ds(cc * 128, 128)] = words[cc]
            b, l0 = (c * nl) // 64, (c * nl) % 64
            for p, f in ((0, _lo), (1, _hi)):
                xs = jnp.concatenate([f(w) for w in words], axis=1)
                xnv = _ln(xs).astype(bf)
                _st(xn, b * 1024 + i * 128 + 64 * (p ^ b) + l0, xnv)
                last["ln"] = _pack(xnv[0:16, 0:128])
                if pin and i == 7 and p == 1:
                    pend.append([pin, _pack(xnv[0:16, 0:128])])
                yield
    N_LN1 = 16

    def mm(p, g, t, nt, i):
        return lax.dot_general(apply_pins(_ld(wt, g * 384 + t * 128, nt * 128), nt),
                               _ld(xn, p * 1024 + i * 128, 128), NT,
                               preferred_element_type=jnp.float32)

    def kv_piece(p, g, i):
        r = mm(p, g, 0, 2, i)
        kvres.append(pltpu.bitcast(r[0:8], jnp.uint32))
        last64 = lax.broadcasted_iota(jnp.int32, (128, 128), 1) % 64 == 63
        for bb, prev, rr in ((kb.at[p * NG + g], kb.at[g], r[:128]), (vb.at[p * NG + g], vb.at[g], r[128:])):
            bb[7 + i] = rr
            if i >= 1:
                if p == 1:
                    rr = jnp.where(last64, prev[7 + i], rr)
                bb[i - 1] = pltpu.roll(rr, 1, 1)

    def q_piece(p, g, i):
        attn_col(p, g, i, mm(p, g, 2, 1, i))

    def q_piece2(p, g, i):
        lhs = jnp.concatenate([_ld(wt, g * 384 + 256, 128), _ld(wt, (g + 1) * 384 + 256, 128)], axis=0)
        qq = lax.dot_general(apply_pins(lhs, 2), _ld(xn, p * 1024 + i * 128, 128), NT,
                             preferred_element_type=jnp.float32)
        attn_col(p, g, i, qq[:128])
        attn_col(p, g + 1, i, qq[128:])

    def attn_col(p, g, i, qv):
        kk, vv = kb.at[p * NG + g], vb.at[p * NG + g]
        lane0 = lax.broadcasted_iota(jnp.int32, (8, 128), 1) % 64 == 0
        acc = [None] * 8
        for d in range(16):
            sl = pl.ds(8 * d, 8)
            q = qv[8 * d:8 * d + 8]
            for w in range(8):
                pr = q * kk[i + 7 - w, sl, :]
                acc[w] = pr if acc[w] is None else acc[w] + pr
        ts = []
        for w in range(8):
            t = acc[w] * (0.25 * LOG2E)
            if w > i and p == 0:
                t = jnp.where(lane0, -1e9 * LOG2E, t)
            ts.append(t)
        mx = jnp.maximum
        m = mx(mx(mx(ts[0], ts[1]), mx(ts[2], ts[3])), mx(mx(ts[4], ts[5]), mx(ts[6], ts[7])))
        ps = [jnp.exp2(t - m) for t in ts]
        ssum = ((ps[0] + ps[1]) + (ps[2] + ps[3])) + ((ps[4] + ps[5]) + (ps[6] + ps[7]))
        r = 1.0 / ssum
        att = [pw * r for pw in ps]
        outs = []
        for d in range(16):
            sl = pl.ds(8 * d, 8)
            prs = [att[w] * vv[i + 7 - w, sl, :] for w in range(8)]
            if TREE == 1:
                outs.append(((prs[0] + prs[1]) + (prs[2] + prs[3])) + ((prs[4] + prs[5]) + (prs[6] + prs[7])))
            elif TREE == 2:
                outs.append((((prs[0] + prs[1]) + prs[2]) + prs[3]) + (((prs[4] + prs[5]) + prs[6]) + prs[7]))
            else:
                outs.append(functools.reduce(lambda a_, b_: a_ + b_, prs))
        blk = _pack(jnp.concatenate(outs, axis=0).T.astype(bf))
        o[g, pl.ds((p * 1024 + i * 128) // 2, 64), :] = blk
        if PINL[p] > 0:
            pend.append([PINL[p], blk[0:8]])

    lane = lax.broadcasted_iota(jnp.int32, (8 * TL, 128), 1)
    GROUPS = ((0, 4), (4, 8), (8, 11))
    ntile = 128 // TL

    def m8(v):
        return v if isinstance(v, int) else pl.multiple_of(v, 8)

    class Tile:
        def __init__(self, p, t):
            self.p, self.t = p, t
            self.acts = {}
            self.y = None

        def wo(self):
            p, t = self.p, self.t
            o_t = jnp.concatenate(
                [jnp.concatenate(
                    [pltpu.bitcast(o[g, pl.ds(m8(p * 512 + i * 64 + 32 * (par ^ p) + 8 * t), 8), :], bf)
                     for g in range(4)], axis=1) for i in range(8) for par in range(2)], axis=0)
            wmat = jnp.concatenate([pltpu.bitcast(wop[c], bf) for c in range(4)], axis=1)
            attn = jnp.dot(apply_pins(o_t, 8), wmat, preferred_element_type=jnp.float32)
            xs = []
            for i in range(8):
                w = xw[i, pl.ds(m8(64 * p + 16 * t), 16), :]
                xs += [_lo(w), _hi(w)]
            h_t = jnp.concatenate(xs, axis=0) + attn
            self.h_t = h_t
            self.hn = _ln(h_t).astype(bf)

        def w1(self, j):
            n = min(128, F - j * 128)
            h1 = lax.dot_general(apply_pins(self.hn, 2), _ld(w1b, j * 128, 128), NT,
                                 preferred_element_type=jnp.float32)
            bj = b1f[:, pl.ds(j * 128, 128)]
            a = _mish((h1.reshape(-1, 8, 128) + bj[None]).reshape(h1.shape))
            if n < 128:
                a = jnp.where(lane < n, a, 0.0)
            self.acts[j] = a.astype(bf)

        def w2(self, gi):
            j0, j1 = GROUPS[gi]
            yj = jnp.dot(apply_pins(jnp.concatenate([self.acts.pop(j) for j in range(j0, j1)], axis=1), 2 * (j1 - j0)),
                         _ld(w2b, j0 * 128, (j1 - j0) * 128), preferred_element_type=jnp.float32)
            self.y = (self.h_t + yj) if self.y is None else self.y + yj

        def fin(self):
            res, p, t = self.y, self.p, self.t
            for i in range(8):
                wds = pltpu.pack_elementwise(
                    [res[32 * i:32 * i + 16], res[32 * i + 16:32 * i + 32]], packed_dtype=bf)
                for cc in range(4):
                    outw[cc, pl.ds(8 * (64 * p + 16 * t) + i, 16, stride=8), :] = wds[:, cc * 128:(cc + 1) * 128]
            for cc in range(4):
                out_copy(4 * p + t, cc).start()

    for t in (1, 2):
        wq_copy(4 * t).wait()
    prep_wt(0, 0)
    prep_wt(0, 1)
    for c in range(NXC // 2):
        z = after(last["ln"]) if (c > 0 and ANCH) else 0
        for cc in range(4):
            x_copy(c, cc, z).wait()
        interleave((ln1_chunk(c), N_LN1))

    P = functools.partial
    units = [(0, 0), (0, 1), (0, 2), (0, 3), (1, 0), (1, 1), (1, 2), (1, 3)]
    kvs = [(P(kv_piece, p, g, i), (p, g)) for (p, g) in units for i in range(8)]
    NA = int(E("NA", 32))
    allq = [(b_, g, i) for b_ in range(2) for g in range(NG) for i in range(8)]
    q0s = [P(q_piece, *u) for u in allq[:NA]]
    if int(E("DQ", 1)):
        q1s = [P(q_piece2, 1, g, i) for i in range(8) for g in (0, 2)]
    else:
        q1s = [P(q_piece, *u) for u in allq[NA:]]
    Q0 = float(E("Q0", 10)); QEND = float(E("QEND", 58))
    LN0 = int(E("LN0", 11)); LNS = float(E("LNS", 4)); LNPIN = int(E("LNPIN", 8))
    kv_done = {}
    for n, (f, u) in enumerate(kvs):
        kv_done[u] = n + 1
    NE = int(E("NE", 1))
    qpos = [9.0] * NE + [max(Q0 + (QEND - Q0) * (j - NE) / (NA - NE - 1.0), kv_done[allq[j][:2]] + 0.5)
                         for j in range(NE, NA)]
    AN = dict(x=int(E("ANX", 6)), g1=int(E("ANG1", 7)), q1=11, g2=12, g3=int(E("ANG3", 20)), ffn=int(E("ANF", 40)))

    def wz(name):
        return after(kvres[AN[name]])

    def w_x():
        z = wz("x")
        for c in range(NXC // 2, NXC):
            for cc in range(4):
                x_copy(c, cc, z).wait()

    def w_g(g, ts, name):
        z = wz(name)
        for t in ts:
            wq_copy(4 * t + g, z).wait()

    def w_g3():
        w_g(3, (1, 2, 0), "g3")
        z = wz("g3")
        for s_ in range(4):
            wo_copy(s_, z).wait()
        interleave((prep_wo(), N_PREP_WO))

    def w_ffn():
        z = wz("ffn")
        b1_copy(z).wait()
        for s_ in range(4):
            w1_copy(s_, z).wait()
            w2_copy(s_, z).wait()
        bv = b1b[...].astype(jnp.float32).reshape(1, F)
        b1f[:, pl.ds(0, 1280)] = jnp.broadcast_to(bv[:, :1280], (8, 1280))
        b1f[:, pl.ds(1280, 128)] = jnp.broadcast_to(
            jnp.concatenate([bv[:, 1280:], jnp.zeros((1, FP - F), jnp.float32)], axis=1), (8, 128))

    hooks = {
        3: [P(w_g, 1, (1, 2), "g1"), P(prep_wt, 1, 0)],
        4: [P(prep_wt, 1, 1)],
        5: [P(w_g, 0, (0,), "q0"), P(w_g, 1, (0,), "q0"), P(prep_wt, 0, 2)],
        10: [w_x, P(prep_wt, 1, 2)],
        12: [P(w_g, 2, (1, 2, 0), "g2"), P(prep_wt, 2, 0)],
        13: [P(prep_wt, 2, 1)],
        15: [P(prep_wt, 2, 2)],
        18: [w_g3, P(prep_wt, 3, 0)],
        20: [P(prep_wt, 3, 1)],
        23: [P(prep_wt, 3, 2)],
        41: [w_ffn],
    }
    AN.update(g1=2, q0=4, x=9, g2=11, g3=17)
    SKIP = [int(v) for v in E('SKIP', '').split(',') if v]
    tiles = [Tile(p, t) for p in range(2) for t in range(ntile) if 4 * p + t not in SKIP]
    WO0 = int(E("WO0", 63))
    nq = 0
    nln = NXC // 2
    for n, (f, u) in enumerate(kvs):
        if n == WO0:
            while nq < NA:
                q0s[nq]()
                nq += 1
            tiles[0].wo()
        for hk in hooks.get(n, []):
            if hk == "q":
                if nq < NA and qpos[nq] <= n:
                    q0s[nq]()
                    nq += 1
            else:
                hk()
        while nln < NXC and LN0 + LNS * (nln - NXC // 2) <= n:
            interleave((ln1_chunk(nln, LNPIN), N_LN1))
            nln += 1
        while nq < NA and qpos[nq] <= n:
            q0s[nq]()
            nq += 1
        f()
    while nq < NA:
        q0s[nq]()
        nq += 1

    def gen(fns):
        for f in fns:
            f()
            yield

    if WO0 >= len(kvs):
        tiles[0].wo()
    nq = 0
    NPRE = int(E("NPRE", 1))
    for _ in range(NPRE):
        if nq < len(q1s):
            q1s[nq](); nq += 1
    PAT0 = E("PAT0", "01234567qAq89XqBqWCF").split(",")
    PAT1 = E("PAT1", "01234567A89XBWCF")
    def run(T, pat, nxt=None):
        nonlocal nq
        for ch in pat:
            if ch == "q":
                if nq < len(q1s):
                    q1s[nq]()
                    nq += 1
            elif ch in "ABC":
                T.w2("ABC".index(ch))
            elif ch == "W":
                nxt.wo()
            elif ch == "F":
                T.fin()
            else:
                T.w1(10 if ch == "X" else int(ch))

    def save_carry(T):
        ybuf[...] = T.y
        for j in (8, 9, 10):
            abuf[j - 8] = _pack(T.acts[j])

    def load_carry(T):
        T.y = ybuf[...]
        for j in (8, 9, 10):
            T.acts[j] = pltpu.bitcast(abuf[j - 8], bf)

    LOOP = int(E("LOOP", 1))
    if not LOOP:
        for n, T in enumerate(tiles):
            pat = PAT0[min(n, len(PAT0) - 1)] if T.p == 0 else PAT1
            if n + 1 == len(tiles):
                pat = pat.replace("W", "")
            run(T, pat, tiles[n + 1] if n + 1 < len(tiles) else None)
    else:
        for n in range(3):
            run(tiles[n], PAT0[min(n, len(PAT0) - 1)], tiles[n + 1])
        head = PAT0[min(3, len(PAT0) - 1)]
        run(tiles[3], head[:head.index("W")])
        save_carry(tiles[3])
        body_pat = PAT1[:PAT1.index("W")]

        @pl.loop(0, 2)
        def _(it):
            tau = 3 + 2 * it
            T = Tile(tau // 4, tau % 4)
            load_carry(T)
            for k in (1, 2):
                U = Tile((tau + k) // 4, (tau + k) % 4)
                run(T, "WCF", U)
                run(U, body_pat)
                T = U
            save_carry(T)

        T = tiles[7]
        load_carry(T)
        run(T, "CF")
    assert nq == len(q1s), nq
    for t in range(2 * ntile):
        for cc in range(4):
            if t not in SKIP:
                out_copy(t, cc).wait()


def build():
    bf, f32 = jnp.bfloat16, jnp.float32
    V = pltpu.VMEM
    u32 = jnp.uint32
    scratch = [
        V((4, S // 2, 128), u32), V((12, D // 2, 128), u32), V((4, D // 2, 128), u32),
        V((4, FP // 2, 128), u32), V((4, FP // 2, 128), u32), V((F,), bf), V((8, FP), f32),
        V((4, S // 2, 128), u32), V((8, 128, D), u32),
        V((64, 128), u32), V((4, 3 * D // 2, 128), u32), V((4, D // 2, 128), u32),
        V((8, 15, 128, 128), f32), V((8, 15, 128, 128), f32), V((4, S // 2, 128), u32), V((4, S // 2, 128), u32),
        V((256, D), f32), V((3, 128, 128), u32), V((48, 64, 128), u32),
        pltpu.SemaphoreType.DMA((57,)),
        pltpu.SemaphoreType.DMA((8, 4)),
        pltpu.SemaphoreType.REGULAR((1,)),
    ]
    return pl.pallas_call(
        kernel,
        out_shape=jax.ShapeDtypeStruct((S, D), bf),
        in_specs=[pl.BlockSpec(memory_space=pl.ANY)] * 6,
        out_specs=pl.BlockSpec(memory_space=pl.ANY),
        scratch_shapes=scratch,
        compiler_params=pltpu.CompilerParams(vmem_limit_bytes=100 * 1024 * 1024, flags=FLAGS, disable_semaphore_checks=True),
        name="fused_block",
    )


_B = None


@jax.jit
def pallas_sequential_preLN__sliding_local_dilated__dense_activation_mish__prompt_kernel(
    A_x, A_wqkv, A_wo, B_x, B_w1, B_b1, B_w2,
):
    del B_x
    out = build()(A_x.reshape(S, D), A_wqkv, A_wo, B_w1.T, B_b1, B_w2)
    return out.reshape(1, S, D)
```

```python
import functools

import jax
import jax.numpy as jnp
from jax import lax
from jax.experimental import pallas as pl
from jax.experimental.pallas import tpu as pltpu

S, D, F, FP = 2048, 512, 1376, 1408
NG = 4
NXC = 8
TL = 32
LOG2E = 1.4426950408889634
EPS = 1e-5
NT = (((1,), (1,)), ((), ()))
GROUPS = ((0, 4), (4, 8), (8, 11))
FLAGS = {'XLA_TPU_RESCHEDULE_DMA_DONES': True}


def _ln(x):
    m = jnp.mean(x, axis=-1, keepdims=True)
    xc = x - m
    v = jnp.mean(xc * xc, axis=-1, keepdims=True)
    return xc * jnp.exp2(-0.5 * jnp.log2(v + EPS))


def _lo(w):
    return pltpu.bitcast(w << 16, jnp.float32)


def _hi(w):
    return pltpu.bitcast(w & jnp.uint32(0xFFFF0000), jnp.float32)


def _mish(h):
    e = jnp.exp2(jnp.minimum(h * LOG2E, 20.0 * LOG2E))
    n = e * (e + 2.0)
    return (h * n) * pl.reciprocal(n + 2.0, approx=True)


def _drain(gen):
    for _ in gen:
        pass


def _pack(v):
    return pltpu.bitcast(v, jnp.uint32)


def _ld(ref, r0, n):
    return jnp.concatenate(
        [pltpu.bitcast(ref[c, pl.ds(r0 // 2, n // 2), :], jnp.bfloat16) for c in range(4)], axis=1)


def _st(ref, r0, v):
    for c in range(4):
        ref[c, pl.ds(r0 // 2, v.shape[0] // 2), :] = _pack(v[:, c * 128:(c + 1) * 128])


def kernel(x_hbm, wqkv_hbm, wo_hbm, w1_hbm, b1_hbm, w2_hbm, out_hbm,
           xbuf, wqb, wob, w1b, w2b, b1b, b1f, xn, xw, pm, wt, wop,
           kb, vb, o, outw, ybuf, abuf, wtmp,
           sem_in, sem_out, zsem):
    RC = S // NXC
    bf = jnp.bfloat16

    zs = pl.semaphore_read(zsem.at[0])
    pend = []
    pin_no = [0]
    kvres = []
    last = {}

    def after(v):
        return pltpu.bitcast(v, jnp.int32)[0, 0] & zs

    def apply_pins(lhs, cost=1):
        for e in pend:
            e[0] -= cost
        due = [e for e in pend if e[0] <= 0]
        for e in due:
            pend.remove(e)
            pin_no[0] += 1
            zv = jnp.full((8, 128), zs * pin_no[0], jnp.int32).astype(jnp.uint32)
            first = pltpu.bitcast(pltpu.bitcast(lhs[0:16, 0:128], jnp.uint32) | (e[1] & zv), lhs.dtype)
            top = jnp.concatenate([first, lhs[0:16, 128:]], axis=1) if lhs.shape[1] > 128 else first
            lhs = jnp.concatenate([top, lhs[16:]], axis=0)
        return lhs

    def x_copy(c, cc, z=0):
        return pltpu.make_async_copy(
            x_hbm.at[pl.ds(c * RC, RC), pl.ds(cc * 128, 128)],
            xbuf.at[cc].bitcast(bf).at[pl.ds(c * RC, RC), :], sem_in.at[z + c * 4 + cc])

    def wq_copy(s, z=0):
        return pltpu.make_async_copy(
            wqkv_hbm.at[:, pl.ds(s * 128, 128)], wqb.at[s].bitcast(bf), sem_in.at[z + 32 + s])

    def wo_copy(s, z=0):
        return pltpu.make_async_copy(
            wo_hbm.at[:, pl.ds(s * 128, 128)], wob.at[s].bitcast(bf), sem_in.at[z + 44 + s])

    def w1_copy(s, z=0):
        return pltpu.make_async_copy(
            w1_hbm.at[:, pl.ds(s * 128, 128)], w1b.at[s].bitcast(bf).at[pl.ds(0, F), :], sem_in.at[z + 48 + s])

    def w2_copy(s, z=0):
        return pltpu.make_async_copy(
            w2_hbm.at[:, pl.ds(s * 128, 128)], w2b.at[s].bitcast(bf).at[pl.ds(0, F), :], sem_in.at[z + 52 + s])

    def b1_copy(z=0):
        return pltpu.make_async_copy(b1_hbm, b1b, sem_in.at[z + 56])

    def out_copy(t, cc):
        r0 = t * 256 if isinstance(t, int) else pl.multiple_of(t * 256, 256)
        return pltpu.make_async_copy(
            outw.at[cc].bitcast(bf).at[pl.ds(r0, 256), :],
            out_hbm.at[pl.ds(r0, 256), pl.ds(cc * 128, 128)], sem_out.at[t, cc])

    for t in (1, 2):
        wq_copy(4 * t).start()
    for c in range(NXC // 2):
        for cc in range(4):
            x_copy(c, cc).start()
    for t in (1, 2, 0):
        wq_copy(4 * t + 1).start()
    wq_copy(0).start()
    for c in range(NXC // 2, NXC):
        for cc in range(4):
            x_copy(c, cc).start()
    for g in range(2, NG):
        for t in (1, 2, 0):
            wq_copy(4 * t + g).start()
    for s in range(4):
        wo_copy(s).start()
    b1_copy().start()
    for s in range(4):
        w1_copy(s).start()
    for s in range(4):
        w2_copy(s).start()

    for s in range(4):
        w1b[s, pl.ds(F // 2, (FP - F) // 2), :] = jnp.zeros(((FP - F) // 2, 128), jnp.uint32)
        w2b[s, pl.ds(F // 2, (FP - F) // 2), :] = jnp.zeros(((FP - F) // 2, 128), jnp.uint32)

    rho = lax.broadcasted_iota(jnp.int32, (128, 128), 0)
    fi = lax.broadcasted_iota(jnp.int32, (128, 128), 1)
    pm[...] = _pack(jnp.where(fi == 16 * (rho % 8) + rho // 8, 1.0, 0.0).astype(bf))

    def prep_wt(g, t):
        s = 4 * ((t + 1) % 3) + g
        r0 = g * 384 + t * 128
        if g == 0 and t < 2:
            r = lax.dot_general(pltpu.bitcast(pm[...], bf), pltpu.bitcast(wqb[s], bf), NT,
                                preferred_element_type=jnp.float32)
            _st(wt, r0, r.astype(bf))
            return
        for dt in range(4):
            tmp = wtmp.at[s * 4 + dt]
            tmp[...] = _pack(pltpu.bitcast(wqb[s, pl.ds(64 * dt, 64), :], bf).T)
            parts = []
            for j in range(8):
                w = tmp[pl.ds(j, 8, stride=8), :]
                parts += [_lo(w), _hi(w)]
            wt[dt, pl.ds(r0 // 2, 64), :] = _pack(jnp.concatenate(parts, axis=0).astype(bf))
            if dt == 3:
                pend.append([6, wt[dt, pl.ds(r0 // 2, 8), :]])

    def prep_wo():
        for s in range(4):
            for g in range(NG):
                parts = []
                for j in range(8):
                    w = wob[s, pl.ds(g * 64 + j, 8, stride=8), :]
                    parts += [_lo(w), _hi(w)]
                wop[s, pl.ds(g * 64, 64), :] = _pack(jnp.concatenate(parts, axis=0).astype(bf))

    def ln1_chunk(c, pin=0):
        nl = RC // 16
        b, l0 = (c * nl) // 64, (c * nl) % 64
        for i in range(8):
            words = [xbuf[cc, pl.ds(c * RC // 2 + i, nl, stride=8), :] for cc in range(4)]
            for cc in range(4):
                xw[i, pl.ds(c * nl, nl), pl.ds(cc * 128, 128)] = words[cc]
            for p, f in ((0, _lo), (1, _hi)):
                xs = jnp.concatenate([f(w) for w in words], axis=1)
                xnv = _ln(xs).astype(bf)
                _st(xn, b * 1024 + i * 128 + 64 * (p ^ b) + l0, xnv)
                last["ln"] = _pack(xnv[0:16, 0:128])
                if pin and i == 7 and p == 1:
                    pend.append([pin, _pack(xnv[0:16, 0:128])])

    def mm(b, g, t, nt, i):
        return lax.dot_general(apply_pins(_ld(wt, g * 384 + t * 128, nt * 128), nt),
                               _ld(xn, b * 1024 + i * 128, 128), NT,
                               preferred_element_type=jnp.float32)

    def kv_piece(b, g, i):
        r = mm(b, g, 0, 2, i)
        kvres.append(pltpu.bitcast(r[0:8], jnp.uint32))
        last64 = lax.broadcasted_iota(jnp.int32, (128, 128), 1) % 64 == 63
        for bb, prev, rr in ((kb.at[b * NG + g], kb.at[g], r[:128]), (vb.at[b * NG + g], vb.at[g], r[128:])):
            bb[7 + i] = rr
            if i >= 1:
                if b == 1:
                    rr = jnp.where(last64, prev[7 + i], rr)
                bb[i - 1] = pltpu.roll(rr, 1, 1)

    def q_piece(b, g, i):
        attn_col(b, g, i, mm(b, g, 2, 1, i))

    def q_piece2(b, g, i):
        lhs = jnp.concatenate([_ld(wt, g * 384 + 256, 128), _ld(wt, (g + 1) * 384 + 256, 128)], axis=0)
        qq = lax.dot_general(apply_pins(lhs, 2), _ld(xn, b * 1024 + i * 128, 128), NT,
                             preferred_element_type=jnp.float32)
        attn_col(b, g, i, qq[:128])
        attn_col(b, g + 1, i, qq[128:])

    def attn_col(b, g, i, qv):
        kk, vv = kb.at[b * NG + g], vb.at[b * NG + g]
        lane0 = lax.broadcasted_iota(jnp.int32, (8, 128), 1) % 64 == 0
        acc = [None] * 8
        for d in range(16):
            sl = pl.ds(8 * d, 8)
            q = qv[8 * d:8 * d + 8]
            for w in range(8):
                pr = q * kk[i + 7 - w, sl, :]
                acc[w] = pr if acc[w] is None else acc[w] + pr
        ts = []
        for w in range(8):
            t = acc[w] * (0.25 * LOG2E)
            if w > i and b == 0:
                t = jnp.where(lane0, -1e9 * LOG2E, t)
            ts.append(t)
        mx = jnp.maximum
        m = mx(mx(mx(ts[0], ts[1]), mx(ts[2], ts[3])), mx(mx(ts[4], ts[5]), mx(ts[6], ts[7])))
        ps = [jnp.exp2(t - m) for t in ts]
        ssum = ((ps[0] + ps[1]) + (ps[2] + ps[3])) + ((ps[4] + ps[5]) + (ps[6] + ps[7]))
        r = 1.0 / ssum
        att = [pw * r for pw in ps]
        outs = []
        for d in range(16):
            sl = pl.ds(8 * d, 8)
            prs = [att[w] * vv[i + 7 - w, sl, :] for w in range(8)]
            outs.append(((prs[0] + prs[1]) + (prs[2] + prs[3])) + ((prs[4] + prs[5]) + (prs[6] + prs[7])))
        blk = _pack(jnp.concatenate(outs, axis=0).T.astype(bf))
        o[g, pl.ds((b * 1024 + i * 128) // 2, 64), :] = blk
        if b == 1:
            pend.append([10, blk[0:8]])

    lane = lax.broadcasted_iota(jnp.int32, (8 * TL, 128), 1)

    def m8(v):
        return v if isinstance(v, int) else pl.multiple_of(v, 8)

    class Tile:
        def __init__(self, b, t):
            self.b, self.t = b, t
            self.acts = {}
            self.y = None

        def wo(self):
            b, t = self.b, self.t
            o_t = jnp.concatenate(
                [jnp.concatenate(
                    [pltpu.bitcast(o[g, pl.ds(m8(b * 512 + i * 64 + 32 * (par ^ b) + 8 * t), 8), :], bf)
                     for g in range(4)], axis=1) for i in range(8) for par in range(2)], axis=0)
            wmat = jnp.concatenate([pltpu.bitcast(wop[c], bf) for c in range(4)], axis=1)
            attn = jnp.dot(apply_pins(o_t, 8), wmat, preferred_element_type=jnp.float32)
            xs = []
            for i in range(8):
                w = xw[i, pl.ds(m8(64 * b + 16 * t), 16), :]
                xs += [_lo(w), _hi(w)]
            self.h = jnp.concatenate(xs, axis=0) + attn
            self.hn = _ln(self.h).astype(bf)

        def w1(self, j):
            n = min(128, F - j * 128)
            h1 = lax.dot_general(apply_pins(self.hn, 2), _ld(w1b, j * 128, 128), NT,
                                 preferred_element_type=jnp.float32)
            bj = b1f[:, pl.ds(j * 128, 128)]
            a = _mish((h1.reshape(-1, 8, 128) + bj[None]).reshape(h1.shape))
            if n < 128:
                a = jnp.where(lane < n, a, 0.0)
            self.acts[j] = a.astype(bf)

        def w2(self, gi):
            j0, j1 = GROUPS[gi]
            a = jnp.concatenate([self.acts.pop(j) for j in range(j0, j1)], axis=1)
            yj = jnp.dot(apply_pins(a, 2 * (j1 - j0)), _ld(w2b, j0 * 128, (j1 - j0) * 128),
                         preferred_element_type=jnp.float32)
            self.y = (self.h + yj) if self.y is None else self.y + yj

        def fin(self):
            res, b, t = self.y, self.b, self.t
            for i in range(8):
                wds = pltpu.pack_elementwise(
                    [res[32 * i:32 * i + 16], res[32 * i + 16:32 * i + 32]], packed_dtype=bf)
                for cc in range(4):
                    outw[cc, pl.ds(8 * (64 * b + 16 * t) + i, 16, stride=8), :] = wds[:, cc * 128:(cc + 1) * 128]
            for cc in range(4):
                out_copy(4 * b + t, cc).start()

    for t in (1, 2):
        wq_copy(4 * t).wait()
    prep_wt(0, 0)
    prep_wt(0, 1)
    for c in range(NXC // 2):
        z = after(last["ln"]) if c > 0 else 0
        for cc in range(4):
            x_copy(c, cc, z).wait()
        ln1_chunk(c)

    P = functools.partial
    kvs = [(b, g, i) for b in range(2) for g in range(NG) for i in range(8)]
    NA, Q0, QEND = 32, 10.0, 58.0
    q0s = [(0, g, i) for g in range(NG) for i in range(8)]
    qpos = [9.0] + [max(Q0 + (QEND - Q0) * (j - 1) / (NA - 2.0), 8 * (q0s[j][1] + 1) + 0.5) for j in range(1, NA)]

    def w_x():
        z = after(kvres[9])
        for c in range(NXC // 2, NXC):
            for cc in range(4):
                x_copy(c, cc, z).wait()

    def w_g(g, ts, anchor):
        z = after(kvres[anchor])
        for t in ts:
            wq_copy(4 * t + g, z).wait()

    def w_g3():
        w_g(3, (1, 2, 0), 17)
        z = after(kvres[17])
        for s in range(4):
            wo_copy(s, z).wait()
        prep_wo()

    def w_ffn():
        z = after(kvres[40])
        b1_copy(z).wait()
        for s in range(4):
            w1_copy(s, z).wait()
            w2_copy(s, z).wait()
        bv = b1b[...].astype(jnp.float32).reshape(1, F)
        b1f[:, pl.ds(0, 1280)] = jnp.broadcast_to(bv[:, :1280], (8, 1280))
        b1f[:, pl.ds(1280, 128)] = jnp.broadcast_to(
            jnp.concatenate([bv[:, 1280:], jnp.zeros((1, FP - F), jnp.float32)], axis=1), (8, 128))

    hooks = {
        3: [P(w_g, 1, (1, 2), 2), P(prep_wt, 1, 0)],
        4: [P(prep_wt, 1, 1)],
        5: [P(w_g, 0, (0,), 4), P(w_g, 1, (0,), 4), P(prep_wt, 0, 2)],
        10: [w_x, P(prep_wt, 1, 2)],
        12: [P(w_g, 2, (1, 2, 0), 11), P(prep_wt, 2, 0)],
        13: [P(prep_wt, 2, 1)],
        15: [P(prep_wt, 2, 2)],
        18: [w_g3, P(prep_wt, 3, 0)],
        20: [P(prep_wt, 3, 1)],
        23: [P(prep_wt, 3, 2)],
        41: [w_ffn],
    }
    tiles = [Tile(b, t) for b in range(2) for t in range(4)]
    nq = 0
    nln = NXC // 2
    for n, u in enumerate(kvs):
        if n == len(kvs) - 1:
            while nq < NA:
                q_piece(*q0s[nq])
                nq += 1
            tiles[0].wo()
        for hk in hooks.get(n, []):
            hk()
        while nln < NXC and 11 + 4 * (nln - NXC // 2) <= n:
            ln1_chunk(nln, 8)
            nln += 1
        while nq < NA and qpos[nq] <= n:
            q_piece(*q0s[nq])
            nq += 1
        kv_piece(*u)

    q1s = [(1, g, i) for i in range(8) for g in (0, 2)]
    nq = 0
    PAT0 = "01234567qAq89XqBqWCF"
    PAT1 = "01234567A89XB"

    def run(T, pat, nxt=None):
        nonlocal nq
        for ch in pat:
            if ch == "q":
                if nq < len(q1s):
                    q_piece2(*q1s[nq])
                    nq += 1
            elif ch in "ABC":
                T.w2("ABC".index(ch))
            elif ch == "W":
                nxt.wo()
            elif ch == "F":
                T.fin()
            else:
                T.w1(10 if ch == "X" else int(ch))

    def save_carry(T):
        ybuf[...] = T.y
        for j in (8, 9, 10):
            abuf[j - 8] = _pack(T.acts[j])

    def load_carry(T):
        T.y = ybuf[...]
        for j in (8, 9, 10):
            T.acts[j] = pltpu.bitcast(abuf[j - 8], bf)

    run(None, "q")
    for n in range(3):
        run(tiles[n], PAT0, tiles[n + 1])
    run(tiles[3], PAT0[:PAT0.index("W")])
    save_carry(tiles[3])

    @pl.loop(0, 2)
    def _(it):
        tau = 3 + 2 * it
        T = Tile(tau // 4, tau % 4)
        load_carry(T)
        for k in (1, 2):
            U = Tile((tau + k) // 4, (tau + k) % 4)
            run(T, "WCF", U)
            run(U, PAT1)
            T = U
        save_carry(T)

    load_carry(tiles[7])
    run(tiles[7], "CF")
    assert nq == len(q1s), nq
    for t in range(8):
        for cc in range(4):
            out_copy(t, cc).wait()


def build():
    bf, f32, u32 = jnp.bfloat16, jnp.float32, jnp.uint32
    V = pltpu.VMEM
    scratch = [
        V((4, S // 2, 128), u32),
        V((12, D // 2, 128), u32),
        V((4, D // 2, 128), u32),
        V((4, FP // 2, 128), u32),
        V((4, FP // 2, 128), u32),
        V((F,), bf),
        V((8, FP), f32),
        V((4, S // 2, 128), u32),
        V((8, 128, D), u32),
        V((64, 128), u32),
        V((4, 3 * D // 2, 128), u32),
        V((4, D // 2, 128), u32),
        V((8, 15, 128, 128), f32),
        V((8, 15, 128, 128), f32),
        V((4, S // 2, 128), u32),
        V((4, S // 2, 128), u32),
        V((256, D), f32),
        V((3, 128, 128), u32),
        V((48, 64, 128), u32),
        pltpu.SemaphoreType.DMA((57,)),
        pltpu.SemaphoreType.DMA((8, 4)),
        pltpu.SemaphoreType.REGULAR((1,)),
    ]
    return pl.pallas_call(
        kernel,
        out_shape=jax.ShapeDtypeStruct((S, D), bf),
        in_specs=[pl.BlockSpec(memory_space=pl.ANY)] * 6,
        out_specs=pl.BlockSpec(memory_space=pl.ANY),
        scratch_shapes=scratch,
        compiler_params=pltpu.CompilerParams(
            vmem_limit_bytes=100 * 1024 * 1024, flags=FLAGS, disable_semaphore_checks=True),
        name="fused_block",
    )


@jax.jit
def pallas_sequential_preLN__sliding_local_dilated__dense_activation_mish__prompt_kernel(
    A_x, A_wqkv, A_wo, B_x, B_w1, B_b1, B_w2,
):
    del B_x
    out = build()(A_x.reshape(S, D), A_wqkv, A_wo, B_w1.T, B_b1, B_w2)
    return out.reshape(1, S, D)
```

```python
import functools

import jax
import jax.numpy as jnp
from jax import lax
from jax.experimental import pallas as pl
from jax.experimental.pallas import tpu as pltpu

S, D, F, FP = 2048, 512, 1376, 1408
NG = 4
TL = 32
LOG2E = 1.4426950408889634
EPS = 1e-5
NT = (((1,), (1,)), ((), ()))
GROUPS = ((0, 4), (4, 8), (8, 11))
FLAGS = {'XLA_TPU_RESCHEDULE_DMA_DONES': True}


def _ln(x):
    m = jnp.mean(x, axis=-1, keepdims=True)
    xc = x - m
    v = jnp.mean(xc * xc, axis=-1, keepdims=True)
    return xc * jnp.exp2(-0.5 * jnp.log2(v + EPS))


def _lo(w):
    return pltpu.bitcast(w << 16, jnp.float32)


def _hi(w):
    return pltpu.bitcast(w & jnp.uint32(0xFFFF0000), jnp.float32)


def _mish(h):
    e = jnp.exp2(jnp.minimum(h * LOG2E, 20.0 * LOG2E))
    n = e * (e + 2.0)
    return (h * n) * pl.reciprocal(n + 2.0, approx=True)


def _drain(gen):
    for _ in gen:
        pass


def _pack(v):
    return pltpu.bitcast(v, jnp.uint32)


def _ld(ref, r0, n):
    return jnp.concatenate(
        [pltpu.bitcast(ref[c, pl.ds(r0 // 2, n // 2), :], jnp.bfloat16) for c in range(4)], axis=1)


def _st(ref, r0, v):
    for c in range(4):
        ref[c, pl.ds(r0 // 2, v.shape[0] // 2), :] = _pack(v[:, c * 128:(c + 1) * 128])


def kernel(x_hbm, wqkv_hbm, wo_hbm, w1_hbm, b1_hbm, w2_hbm, out_hbm,
           xbuf, wqb, wob, w1b, w2b, b1b, b1f, xn, xw, pm, wt, wop,
           kb, vb, o, outw, ybuf, abuf, wtmp,
           sem_in, sem_out, zsem):
    bf = jnp.bfloat16

    zs = pl.semaphore_read(zsem.at[0])
    pend = []
    pin_no = [0]
    kvres = []

    def after(v):
        return pltpu.bitcast(v, jnp.int32)[0, 0] & zs

    def apply_pins(lhs, cost=1):
        for e in pend:
            e[0] -= cost
        due = [e for e in pend if e[0] <= 0]
        for e in due:
            pend.remove(e)
            pin_no[0] += 1
            zv = jnp.full((8, 128), zs * pin_no[0], jnp.int32).astype(jnp.uint32)
            first = pltpu.bitcast(pltpu.bitcast(lhs[0:16, 0:128], jnp.uint32) | (e[1] & zv), lhs.dtype)
            top = jnp.concatenate([first, lhs[0:16, 128:]], axis=1) if lhs.shape[1] > 128 else first
            lhs = jnp.concatenate([top, lhs[16:]], axis=0)
        return lhs

    def x_copy(b, k, cc, z=0):
        r0, nr = (4 * k, 4) if b == 0 else (0, 16)
        return pltpu.make_async_copy(
            x_hbm.at[pl.ds(64 * b, 64), pl.ds(r0, nr), pl.ds(cc * 128, 128)],
            xbuf.at[cc, pl.ds(64 * b, 64)].bitcast(bf).at[:, pl.ds(r0, nr), :],
            sem_in.at[z + (7 * b + k) * 4 + cc])

    def wq_copy(s, z=0):
        return pltpu.make_async_copy(
            wqkv_hbm.at[:, pl.ds(s * 128, 128)], wqb.at[s].bitcast(bf), sem_in.at[z + 32 + s])

    def wo_copy(s, z=0):
        return pltpu.make_async_copy(
            wo_hbm.at[:, pl.ds(s * 128, 128)], wob.at[s].bitcast(bf), sem_in.at[z + 44 + s])

    def w1_copy(s, z=0):
        return pltpu.make_async_copy(
            w1_hbm.at[:, pl.ds(s * 128, 128)], w1b.at[s].bitcast(bf).at[pl.ds(0, F), :], sem_in.at[z + 48 + s])

    def w2_copy(s, z=0):
        return pltpu.make_async_copy(
            w2_hbm.at[:, pl.ds(s * 128, 128)], w2b.at[s].bitcast(bf).at[pl.ds(0, F), :], sem_in.at[z + 52 + s])

    def b1_copy(z=0):
        return pltpu.make_async_copy(b1_hbm, b1b, sem_in.at[z + 56])

    def out_copy(t, cc):
        r0 = t * 256 if isinstance(t, int) else pl.multiple_of(t * 256, 256)
        return pltpu.make_async_copy(
            outw.at[cc].bitcast(bf).at[pl.ds(r0, 256), :],
            out_hbm.at[pl.ds(r0, 256), pl.ds(cc * 128, 128)], sem_out.at[t, cc])

    for t in (1, 2):
        wq_copy(4 * t).start()
    for cc in range(4):
        x_copy(0, 0, cc).start()
    for t in (1, 2):
        wq_copy(4 * t + 1).start()
    for k in range(1, 4):
        for cc in range(4):
            x_copy(0, k, cc).start()
    wq_copy(0).start()
    wq_copy(1).start()
    for t in (1, 2, 0):
        wq_copy(4 * t + 2).start()
    for cc in range(4):
        x_copy(1, 0, cc).start()
    for t in (1, 2, 0):
        wq_copy(4 * t + 3).start()
    for s in range(4):
        wo_copy(s).start()
    b1_copy().start()
    for s in range(4):
        w1_copy(s).start()
    for s in range(4):
        w2_copy(s).start()

    for s in range(4):
        w1b[s, pl.ds(F // 2, (FP - F) // 2), :] = jnp.zeros(((FP - F) // 2, 128), jnp.uint32)
        w2b[s, pl.ds(F // 2, (FP - F) // 2), :] = jnp.zeros(((FP - F) // 2, 128), jnp.uint32)

    rho = lax.broadcasted_iota(jnp.int32, (128, 128), 0)
    fi = lax.broadcasted_iota(jnp.int32, (128, 128), 1)
    pm[...] = _pack(jnp.where(fi == 16 * (rho % 8) + rho // 8, 1.0, 0.0).astype(bf))

    def prep_wt(g, t):
        s = 4 * ((t + 1) % 3) + g
        r0 = g * 384 + t * 128
        if g == 0 and t < 2:
            r = lax.dot_general(pltpu.bitcast(pm[...], bf), pltpu.bitcast(wqb[s], bf), NT,
                                preferred_element_type=jnp.float32)
            _st(wt, r0, r.astype(bf))
            return
        for dt in range(4):
            tmp = wtmp.at[s * 4 + dt]
            tmp[...] = _pack(pltpu.bitcast(wqb[s, pl.ds(64 * dt, 64), :], bf).T)
            parts = []
            for j in range(8):
                w = tmp[pl.ds(j, 8, stride=8), :]
                parts += [_lo(w), _hi(w)]
            wt[dt, pl.ds(r0 // 2, 64), :] = _pack(jnp.concatenate(parts, axis=0).astype(bf))
            if dt == 3:
                pend.append([6, wt[dt, pl.ds(r0 // 2, 8), :]])

    def prep_wo():
        for s in range(4):
            for g in range(NG):
                parts = []
                for j in range(8):
                    w = wob[s, pl.ds(g * 64 + j, 8, stride=8), :]
                    parts += [_lo(w), _hi(w)]
                wop[s, pl.ds(g * 64, 64), :] = _pack(jnp.concatenate(parts, axis=0).astype(bf))

    def ln1_tile(b, i, pin=0):
        words = [xbuf.at[cc].reshape(S // 2, 128)[pl.ds(512 * b + i, 64, stride=8), :] for cc in range(4)]
        for cc in range(4):
            xw[i, pl.ds(64 * b, 64), pl.ds(cc * 128, 128)] = words[cc]
        for p, f in ((0, _lo), (1, _hi)):
            xs = jnp.concatenate([f(w) for w in words], axis=1)
            xnv = _ln(xs).astype(bf)
            _st(xn, b * 1024 + i * 128 + 64 * (p ^ b), xnv)
            if pin and p == 1:
                pend.append([pin, _pack(xnv[0:16, 0:128])])

    def mm(b, g, t, nt, i):
        return lax.dot_general(apply_pins(_ld(wt, g * 384 + t * 128, nt * 128), nt),
                               _ld(xn, b * 1024 + i * 128, 128), NT,
                               preferred_element_type=jnp.float32)

    def kv_piece(b, g, i):
        r = mm(b, g, 0, 2, i)
        kvres.append(pltpu.bitcast(r[0:8], jnp.uint32))
        last64 = lax.broadcasted_iota(jnp.int32, (128, 128), 1) % 64 == 63
        for bb, prev, rr in ((kb.at[b * NG + g], kb.at[g], r[:128]), (vb.at[b * NG + g], vb.at[g], r[128:])):
            bb[7 + i] = rr
            if i >= 1:
                if b == 1:
                    rr = jnp.where(last64, prev[7 + i], rr)
                bb[i - 1] = pltpu.roll(rr, 1, 1)

    def q_piece(b, g, i):
        attn_col(b, g, i, mm(b, g, 2, 1, i))

    def q_piece2(b, g, i):
        lhs = jnp.concatenate([_ld(wt, g * 384 + 256, 128), _ld(wt, (g + 1) * 384 + 256, 128)], axis=0)
        qq = lax.dot_general(apply_pins(lhs, 2), _ld(xn, b * 1024 + i * 128, 128), NT,
                             preferred_element_type=jnp.float32)
        attn_col(b, g, i, qq[:128])
        attn_col(b, g + 1, i, qq[128:])

    def attn_col(b, g, i, qv):
        kk, vv = kb.at[b * NG + g], vb.at[b * NG + g]
        lane0 = lax.broadcasted_iota(jnp.int32, (8, 128), 1) % 64 == 0
        acc = [None] * 8
        for d in range(16):
            sl = pl.ds(8 * d, 8)
            q = qv[8 * d:8 * d + 8]
            for w in range(8):
                pr = q * kk[i + 7 - w, sl, :]
                acc[w] = pr if acc[w] is None else acc[w] + pr
        ts = []
        for w in range(8):
            t = acc[w] * (0.25 * LOG2E)
            if w > i and b == 0:
                t = jnp.where(lane0, -1e9 * LOG2E, t)
            ts.append(t)
        mx = jnp.maximum
        m = mx(mx(mx(ts[0], ts[1]), mx(ts[2], ts[3])), mx(mx(ts[4], ts[5]), mx(ts[6], ts[7])))
        ps = [jnp.exp2(t - m) for t in ts]
        ssum = ((ps[0] + ps[1]) + (ps[2] + ps[3])) + ((ps[4] + ps[5]) + (ps[6] + ps[7]))
        r = 1.0 / ssum
        att = [pw * r for pw in ps]
        outs = []
        for d in range(16):
            sl = pl.ds(8 * d, 8)
            prs = [att[w] * vv[i + 7 - w, sl, :] for w in range(8)]
            outs.append(((prs[0] + prs[1]) + (prs[2] + prs[3])) + ((prs[4] + prs[5]) + (prs[6] + prs[7])))
        blk = _pack(jnp.concatenate(outs, axis=0).T.astype(bf))
        o[g, pl.ds((b * 1024 + i * 128) // 2, 64), :] = blk
        if b == 1:
            pend.append([10, blk[0:8]])

    lane = lax.broadcasted_iota(jnp.int32, (8 * TL, 128), 1)

    def m8(v):
        return v if isinstance(v, int) else pl.multiple_of(v, 8)

    class Tile:
        def __init__(self, b, t):
            self.b, self.t = b, t
            self.acts = {}
            self.y = None

        def wo(self):
            b, t = self.b, self.t
            o_t = jnp.concatenate(
                [jnp.concatenate(
                    [pltpu.bitcast(o[g, pl.ds(m8(b * 512 + i * 64 + 32 * (par ^ b) + 8 * t), 8), :], bf)
                     for g in range(4)], axis=1) for i in range(8) for par in range(2)], axis=0)
            wmat = jnp.concatenate([pltpu.bitcast(wop[c], bf) for c in range(4)], axis=1)
            attn = jnp.dot(apply_pins(o_t, 8), wmat, preferred_element_type=jnp.float32)
            xs = []
            for i in range(8):
                w = xw[i, pl.ds(m8(64 * b + 16 * t), 16), :]
                xs += [_lo(w), _hi(w)]
            self.h = jnp.concatenate(xs, axis=0) + attn
            self.hn = _ln(self.h).astype(bf)

        def w1(self, j):
            n = min(128, F - j * 128)
            h1 = lax.dot_general(apply_pins(self.hn, 2), _ld(w1b, j * 128, 128), NT,
                                 preferred_element_type=jnp.float32)
            bj = b1f[:, pl.ds(j * 128, 128)]
            a = _mish((h1.reshape(-1, 8, 128) + bj[None]).reshape(h1.shape))
            if n < 128:
                a = jnp.where(lane < n, a, 0.0)
            self.acts[j] = a.astype(bf)

        def w2(self, gi):
            j0, j1 = GROUPS[gi]
            a = jnp.concatenate([self.acts.pop(j) for j in range(j0, j1)], axis=1)
            yj = jnp.dot(apply_pins(a, 2 * (j1 - j0)), _ld(w2b, j0 * 128, (j1 - j0) * 128),
                         preferred_element_type=jnp.float32)
            self.y = (self.h + yj) if self.y is None else self.y + yj

        def fin(self):
            res, b, t = self.y, self.b, self.t
            for i in range(8):
                wds = pltpu.pack_elementwise(
                    [res[32 * i:32 * i + 16], res[32 * i + 16:32 * i + 32]], packed_dtype=bf)
                for cc in range(4):
                    outw[cc, pl.ds(8 * (64 * b + 16 * t) + i, 16, stride=8), :] = wds[:, cc * 128:(cc + 1) * 128]
            for cc in range(4):
                out_copy(4 * b + t, cc).start()

        def w2_fin(self):
            j0, j1 = GROUPS[2]
            b, t = self.b, self.t
            a = jnp.concatenate([self.acts.pop(j) for j in range(j0, j1)], axis=1)
            for cc in range(4):
                wcc = pltpu.bitcast(w2b[cc, pl.ds(j0 * 64, (j1 - j0) * 64), :], bf)
                res = self.y[:, cc * 128:(cc + 1) * 128] + jnp.dot(a, wcc, preferred_element_type=jnp.float32)
                for i in range(8):
                    outw[cc, pl.ds(8 * (64 * b + 16 * t) + i, 16, stride=8), :] = pltpu.pack_elementwise(
                        [res[32 * i:32 * i + 16], res[32 * i + 16:32 * i + 32]], packed_dtype=bf)
                out_copy(4 * b + t, cc).start()

    for t in (1, 2):
        wq_copy(4 * t).wait()
    prep_wt(0, 0)
    prep_wt(0, 1)
    for cc in range(4):
        x_copy(0, 0, cc).wait()
    ln1_tile(0, 0)

    P = functools.partial
    kvs = [(b, g, i) for b in range(2) for g in range(NG) for i in range(8)]
    kvs[:16] = [(0, g, i0 + d) for i0 in range(0, 8, 2) for g in (0, 1) for d in range(2)]
    kv_done = {u[:2]: n + 1 for n, u in enumerate(kvs)}
    NA, Q0, QEND = 32, 18.0, 58.0
    q0s = [(0, g, i) for g in range(NG) for i in range(8)]
    qpos = [max(Q0 + (QEND - Q0) * j / (NA - 1.0), kv_done[q0s[j][:2]] + 0.5) for j in range(NA)]

    def w_x(b, k, anchor):
        z = after(kvres[anchor])
        for cc in range(4):
            x_copy(b, k, cc, z).wait()

    def w_g(g, ts, anchor):
        z = after(kvres[anchor])
        for t in ts:
            wq_copy(4 * t + g, z).wait()

    def w_wo():
        z = after(kvres[25])
        for s in range(4):
            wo_copy(s, z).wait()
        prep_wo()

    def w_ffn():
        z = after(kvres[39])
        b1_copy(z).wait()
        for s in range(4):
            w1_copy(s, z).wait()
            w2_copy(s, z).wait()
        bv = b1b[...].astype(jnp.float32).reshape(1, F)
        b1f[:, pl.ds(0, 1280)] = jnp.broadcast_to(bv[:, :1280], (8, 1280))
        b1f[:, pl.ds(1280, 128)] = jnp.broadcast_to(
            jnp.concatenate([bv[:, 1280:], jnp.zeros((1, FP - F), jnp.float32)], axis=1), (8, 128))

    hooks = {
        0: [P(ln1_tile, 0, 1)],
        2: [P(w_g, 1, (1, 2), 1), P(prep_wt, 1, 0), P(prep_wt, 1, 1)],
        3: [P(w_x, 0, 1, 1), P(ln1_tile, 0, 2)],
        4: [P(ln1_tile, 0, 3)],
        7: [P(w_x, 0, 2, 4), P(ln1_tile, 0, 4)],
        8: [P(ln1_tile, 0, 5)],
        11: [P(w_x, 0, 3, 8), P(ln1_tile, 0, 6)],
        12: [P(ln1_tile, 0, 7), P(w_g, 2, (1, 2, 0), 11), P(prep_wt, 2, 0)],
        13: [P(w_g, 0, (0,), 12), P(w_g, 1, (0,), 12), P(prep_wt, 0, 2), P(prep_wt, 2, 1)],
        14: [P(prep_wt, 1, 2)],
        15: [P(prep_wt, 2, 2)],
        18: [P(w_x, 1, 0, 17)],
        20: [P(w_g, 3, (1, 2, 0), 19), P(prep_wt, 3, 0)],
        21: [P(prep_wt, 3, 1)],
        24: [P(prep_wt, 3, 2)],
        26: [w_wo],
        41: [w_ffn],
    }
    tiles = [Tile(b, t) for b in range(2) for t in range(4)]
    nq = 0
    nln = 0
    for n, u in enumerate(kvs):
        if n == len(kvs) - 1:
            while nq < NA:
                q_piece(*q0s[nq])
                nq += 1
            tiles[0].wo()
        for hk in hooks.get(n, []):
            hk()
        while nln < 8 and 19 + 1.5 * nln <= n:
            ln1_tile(1, nln, 8)
            nln += 1
        while nq < NA and qpos[nq] <= n:
            q_piece(*q0s[nq])
            nq += 1
        kv_piece(*u)

    q1s = [(1, g, i) for i in range(8) for g in (0, 2)]
    nq = 0
    PAT0 = "01234567qAq89XqBqWCF"
    PAT1 = "01234567A89XB"

    def run(T, pat, nxt=None):
        nonlocal nq
        for ch in pat:
            if ch == "q":
                if nq < len(q1s):
                    q_piece2(*q1s[nq])
                    nq += 1
            elif ch in "ABC":
                T.w2("ABC".index(ch))
            elif ch == "W":
                nxt.wo()
            elif ch == "F":
                T.fin()
            else:
                T.w1(10 if ch == "X" else int(ch))

    def save_carry(T):
        ybuf[...] = T.y
        for j in (8, 9, 10):
            abuf[j - 8] = _pack(T.acts[j])

    def load_carry(T):
        T.y = ybuf[...]
        for j in (8, 9, 10):
            T.acts[j] = pltpu.bitcast(abuf[j - 8], bf)

    run(None, "q")
    for n in range(3):
        run(tiles[n], PAT0, tiles[n + 1])
    run(tiles[3], PAT0[:PAT0.index("W")])
    save_carry(tiles[3])

    @pl.loop(0, 2)
    def _(it):
        tau = 3 + 2 * it
        T = Tile(tau // 4, tau % 4)
        load_carry(T)
        for k in (1, 2):
            U = Tile((tau + k) // 4, (tau + k) % 4)
            run(T, "WCF", U)
            run(U, PAT1)
            T = U
        save_carry(T)

    load_carry(tiles[7])
    tiles[7].w2_fin()
    assert nq == len(q1s), nq
    for t in range(8):
        for cc in range(4):
            out_copy(t, cc).wait()


def build():
    bf, f32, u32 = jnp.bfloat16, jnp.float32, jnp.uint32
    V = pltpu.VMEM
    scratch = [
        V((4, 128, 8, 128), u32),
        V((12, D // 2, 128), u32),
        V((4, D // 2, 128), u32),
        V((4, FP // 2, 128), u32),
        V((4, FP // 2, 128), u32),
        V((F,), bf),
        V((8, FP), f32),
        V((4, S // 2, 128), u32),
        V((8, 128, D), u32),
        V((64, 128), u32),
        V((4, 3 * D // 2, 128), u32),
        V((4, D // 2, 128), u32),
        V((8, 15, 128, 128), f32),
        V((8, 15, 128, 128), f32),
        V((4, S // 2, 128), u32),
        V((4, S // 2, 128), u32),
        V((256, D), f32),
        V((3, 128, 128), u32),
        V((48, 64, 128), u32),
        pltpu.SemaphoreType.DMA((57,)),
        pltpu.SemaphoreType.DMA((8, 4)),
        pltpu.SemaphoreType.REGULAR((1,)),
    ]
    return pl.pallas_call(
        kernel,
        out_shape=jax.ShapeDtypeStruct((S, D), bf),
        in_specs=[pl.BlockSpec(memory_space=pl.ANY)] * 6,
        out_specs=pl.BlockSpec(memory_space=pl.ANY),
        scratch_shapes=scratch,
        compiler_params=pltpu.CompilerParams(
            vmem_limit_bytes=100 * 1024 * 1024, flags=FLAGS, disable_semaphore_checks=True),
        name="fused_block",
    )


@jax.jit
def pallas_sequential_preLN__sliding_local_dilated__dense_activation_mish__prompt_kernel(
    A_x, A_wqkv, A_wo, B_x, B_w1, B_b1, B_w2,
):
    del B_x
    out = build()(A_x.reshape(128, 16, D), A_wqkv, A_wo, B_w1.T, B_b1, B_w2)
    return out.reshape(1, S, D)
```
